```python
import jax
import jax.numpy as jnp

def _softmax(x, axis=-1):
    return jax.nn.softmax(x, axis=axis)
def _gelu(x):
    return jax.nn.gelu(x, approximate=True)
def _silu(x):
    return jax.nn.silu(x)
def _sigmoid(x):
    return jax.nn.sigmoid(x)
def _layernorm(x, axis=-1, eps=1e-5):
    m = jnp.mean(x, axis=axis, keepdims=True)
    v = jnp.var(x, axis=axis, keepdims=True)
    return (x - m) / jnp.sqrt(v + eps)
def _scatter_add(tgt, idx, src, axis=0):
    return tgt.at[idx].add(src)
def _segment_sum(src, seg, n):
    return jax.ops.segment_sum(src, seg, n)
class _Rng:
    def __init__(self, key):
        self._k = key
    def _next(self):
        self._k, sub = jax.random.split(self._k)
        return sub
    def normal(self, shape):
        return jax.random.normal(self._next(), shape, dtype=jnp.bfloat16)
    def randint(self, lo, hi, shape):
        return jax.random.randint(self._next(), shape, lo, hi, dtype=jnp.int32)
    def uniform(self, shape, lo=0.0, hi=1.0):
        return jax.random.uniform(self._next(), shape, jnp.bfloat16, lo, hi)
    def permutation(self, n):
        return jax.random.permutation(self._next(), n)


kernel_name = 'sequential_preLN__sliding_local_dilated__moe_arch_mod__prompt'

def setup_inputs():
    _rng = _Rng(jax.random.key(int.from_bytes(__import__("os").urandom(4), "little")))
    _w = (lambda a: (lambda t: t.astype(jnp.bfloat16) if jnp.issubdtype(t.dtype, jnp.floating) else t)(jnp.asarray(a)))
    def _A_setup():
        B, S, D = 1, 2048, 640
        return {
            "x": _w((lambda *s: _rng.normal(s) * 0.05)(B, S, D)),
            "wqkv": _w((lambda *s: _rng.normal(s) * 0.05)(D, 3 * D)),
            "wo": _w((lambda *s: _rng.normal(s) * 0.05)(D, D)),
        }
    _A_in = _A_setup()

    def _B_setup():
        B, S, D, F, C = 1, 2048, 640, 1536, 1
        return {
            "x": _w((lambda *s: _rng.normal(s) * 0.05)(B, S, D)),
            "w_r": _w((lambda *s: _rng.normal(s) * 0.05)(D)),
            "w_gate": _w((lambda *s: _rng.normal(s) * 0.05)(D, F)),
            "w_up": _w((lambda *s: _rng.normal(s) * 0.05)(D, F)),
            "w_down": _w((lambda *s: _rng.normal(s) * 0.05)(F, D)),
        }
    _B_in = _B_setup()

    return {
        "A_x": _A_in["x"],
        "A_wqkv": _A_in["wqkv"],
        "A_wo": _A_in["wo"],
        "B_x": _B_in["x"],
        "B_w_r": _B_in["w_r"],
        "B_w_gate": _B_in["w_gate"],
        "B_w_up": _B_in["w_up"],
        "B_w_down": _B_in["w_down"],
    }

def reference(A_x, A_wqkv, A_wo, B_x, B_w_r, B_w_gate, B_w_up, B_w_down):
    def _A_ref(x, wqkv, wo):
        B, S, D = x.shape
        H = 32; Dh = D // H
        W, dil = 8, 2
        qkv = (lambda x, *d: x.transpose(*d))((x @ wqkv).reshape(B, S, 3, H, Dh), 2, 0, 3, 1, 4)
        q, k, v = qkv[0], qkv[1], qkv[2]
        scale = Dh ** -0.5
        pos = jnp.arange(S)
        off = jnp.arange(W) * dil
        idx = pos[:, None] - off[None, :]
        mask = idx >= 0
        idx_c = jnp.where(mask, idx, 0).reshape(-1)
        kg = k[:, :, idx_c, :].reshape(B, H, S, W, Dh)
        vg = v[:, :, idx_c, :].reshape(B, H, S, W, Dh)
        logits = jnp.einsum("bhsd,bhswd->bhsw", q, kg) * scale
        logits = jnp.where(mask[None, None, :, :], logits, -1e9)
        attn = _softmax(logits, axis=-1)
        o = jnp.einsum("bhsw,bhswd->bhsd", attn, vg)
        return (lambda x, *d: x.transpose(*d))(o, 0, 2, 1, 3).reshape(B, S, D) @ wo

    def _B_ref(x, w_r, w_gate, w_up, w_down):
        B, S, D = x.shape
        C = 1
        r = x @ w_r
        idx = jnp.argsort(-r, axis=-1)[:, :C]
        idx_e = jnp.repeat(idx.reshape(B, C, 1), D, axis=2)
        x_sel = jnp.take_along_axis(x, idx_e, axis=1)
        g = _silu(x_sel @ w_gate)
        u = x_sel @ w_up
        y = (g * u) @ w_down
        r_sel = _sigmoid(jnp.take_along_axis(r, idx, axis=1))
        y = y * r_sel.reshape(B, C, 1)
        b_off = (jnp.arange(B) * S).reshape(B, 1)
        flat_idx = (idx + b_off).reshape(B * C)
        zero = (x * 0.0).reshape(B * S, D)
        upd = _scatter_add(zero, flat_idx, y.reshape(B * C, D), axis=0)
        return x + upd.reshape(B, S, D)

    x = A_x
    h = x + _A_ref(_layernorm(x, axis=-1), A_wqkv, A_wo)
    h2 = h + _B_ref(_layernorm(h, axis=-1), B_w_r, B_w_gate, B_w_up, B_w_down)
    return h2
```

```python
import functools
import jax
import jax.numpy as jnp
import numpy as np
from jax import lax
from jax.experimental import pallas as pl
from jax.experimental.pallas import tpu as pltpu

D, F = 640, 1536
H, DH, W, DIL = 32, 20, 8, 2
NC = D // 128
HALO = 16
F32 = jnp.float32
BF16 = jnp.bfloat16
I32 = jnp.int32
LOG2E = 1.4426950408889634
QSCALE = float(DH ** -0.5) * LOG2E
NEG = -1e9 * LOG2E
EPS = 1e-5


def _cat(xs, axis):
    return xs[0] if len(xs) == 1 else jnp.concatenate(xs, axis=axis)


def _regroup(src_ref, c, dp):
    a = src_ref[c, pl.ds(dp, 16, stride=20), :]
    b = src_ref[c, pl.ds(10 + dp, 16, stride=20), :]
    lo = jnp.bitwise_or(jnp.bitwise_and(a, 0xFFFF), jnp.left_shift(b, 16))
    hi = jnp.bitwise_or(lax.shift_right_logical(a, 16), jnp.bitwise_and(b, -65536))
    return lo, hi


def _bf(x):
    return pltpu.bitcast(x, BF16)


def _i32(x):
    return pltpu.bitcast(x, I32)


def run_interleaved(streams):
    active = []
    pending = sorted(streams, key=lambda t: t[0])
    tick = 0
    while pending or active:
        while pending and pending[0][0] <= tick:
            active.append(pending.pop(0))
        active.sort(key=lambda t: t[2])
        nxt = []
        for item in active:
            try:
                next(item[1])
                nxt.append(item)
            except StopIteration:
                pass
        active = nxt
        tick += 1


def make_kernel(S=2048, TM=256, nsplit=3, mm_off=0, ln2_off=8, order=(0, 1, 2, 3, 4), dbg=None):
    T = S // TM
    NG = TM // 8
    NJ = TM // 16

    def kern(x_hbm, wqkv_hbm, wo_hbm, wr_ref, wg_hbm, wu_hbm, wd_hbm, out_hbm,
             x_v, wraw, woraw, t32, wtp, wop, xn_v, q_v, k_v, v_v, o_v, att_v, hn_v, out_v,
             wg_v, wu_v, wd_v, best_v, patch_v, sem_x, sem_w, sem_f, sem_o, sem_p):
        def x_copy(t):
            return pltpu.make_async_copy(x_hbm.at[pl.ds(t * TM, TM), :], x_v.at[pl.ds(t * TM, TM), :], sem_x.at[t])

        def w_copy(p):
            return pltpu.make_async_copy(wqkv_hbm.at[:, pl.ds(p * D, D)], wraw.at[p], sem_w.at[p])

        def wo_copy():
            return pltpu.make_async_copy(wo_hbm, woraw, sem_w.at[3])

        def f_copies():
            return [pltpu.make_async_copy(wg_hbm, wg_v, sem_f.at[0]),
                    pltpu.make_async_copy(wu_hbm, wu_v, sem_f.at[1]),
                    pltpu.make_async_copy(wd_hbm, wd_v, sem_f.at[2])]

        def o_copy(t):
            return pltpu.make_async_copy(out_v.at[pl.ds(t * TM, TM), :], out_hbm.at[pl.ds(t * TM, TM), :], sem_o.at[t])

        x_copy(0).start()
        for p in (1, 2, 0):
            w_copy(p).start()
        x_copy(1).start()
        wo_copy().start()
        for t in range(2, T):
            x_copy(t).start()

        zeros = jnp.zeros((HALO, 128), F32)
        for c in range(NC):
            k_v[c, pl.ds(0, HALO), :] = zeros
            v_v[c, pl.ds(0, HALO), :] = zeros
        best_v[0] = jnp.full((8, 128), -jnp.inf, F32)
        best_v[1] = jnp.zeros((8, 128), F32)

        def prep_w(p):
            w_copy(p).wait()
            for kt in range(NC):
                for ft in range(NC):
                    tile = wraw[p, pl.ds(kt * 128, 128), pl.ds(ft * 128, 128)]
                    t32[p * NC + kt, pl.ds(64 * ft, 64), :] = _i32(tile.T)
            for kt in range(NC):
                for dp in range(10):
                    lo, hi = _regroup(t32, p * NC + kt, dp)
                    wtp[kt, pl.ds(p * 320 + 32 * dp, 16), :] = lo
                    wtp[kt, pl.ds(p * 320 + 32 * dp + 16, 16), :] = hi

        def prep_wo():
            wo_copy().wait()
            for c in range(NC):
                t32[3 * NC + c] = _i32(woraw[:, pl.ds(c * 128, 128)])
            for c in range(NC):
                for dp in range(10):
                    lo, hi = _regroup(t32, 3 * NC + c, dp)
                    wop[c, pl.ds(32 * dp, 16), :] = lo
                    wop[c, pl.ds(32 * dp + 16, 16), :] = hi

        def ln1_task(r):
            xf = x_v[pl.ds(r, 16), :].astype(F32)
            m = jnp.sum(xf, axis=-1, keepdims=True) * (1.0 / D)
            yield
            xc = xf - m
            v = jnp.sum(xc * xc, axis=-1, keepdims=True) * (1.0 / D)
            yield
            xn = (xc * lax.rsqrt(v + EPS)).astype(BF16)
            for c in range(NC):
                xn_v[c, pl.ds(r // 2, 8), :] = _i32(xn[:, c * 128:(c + 1) * 128])

        NCH = 15 // nsplit

        def qkv_task(t, n):
            r = t * TM
            lhs = _cat([_bf(xn_v[c, pl.ds(r // 2, TM // 2), :]) for c in range(NC)], 1)
            rhs = _cat([_bf(wtp[c, pl.ds(n * nsplit * 64, nsplit * 64), :]) for c in range(NC)], 1)
            y = lax.dot_general(lhs, rhs, (((1,), (1,)), ((), ())), preferred_element_type=F32)
            for i in range(nsplit):
                nt = n * nsplit + i
                p, c = divmod(nt, NC)
                yc = y[:, i * 128:(i + 1) * 128]
                if p == 0:
                    q_v[c, pl.ds(r, TM), :] = yc * QSCALE
                elif p == 1:
                    k_v[c, pl.ds(HALO + r, TM), :] = yc
                else:
                    v_v[c, pl.ds(HALO + r, TM), :] = yc
            yield

        def attn_task(r):
            q = [q_v[c, pl.ds(r, 8), :] for c in range(NC)]
            s = []
            for w in range(W):
                acc = None
                for c in range(NC):
                    pr = q[c] * k_v[c, pl.ds(HALO + r - DIL * w, 8), :]
                    acc = pr if acc is None else acc + pr
                s.append(acc)
            rr = [pltpu.roll(a, 64, 1) for a in s]
            yield
            s = [a + b for a, b in zip(s, rr)]
            rr = [pltpu.roll(a, 32, 1) for a in s]
            yield
            s = [a + b for a, b in zip(s, rr)]
            for w in range(W):
                if r < DIL * w:
                    rows = r + lax.broadcasted_iota(I32, (8, 128), 0)
                    s[w] = jnp.where(rows >= DIL * w, s[w], NEG)
            m = s[0]
            for w in range(1, W):
                m = jnp.maximum(m, s[w])
            p = [jnp.exp2(s[w] - m) for w in range(W)]
            l = p[0]
            for w in range(1, W):
                l = l + p[w]
            inv = 1.0 / l
            for c in range(NC):
                acc = None
                for w in range(W):
                    pr = p[w] * v_v[c, pl.ds(HALO + r - DIL * w, 8), :]
                    acc = pr if acc is None else acc + pr
                o_v[c, pl.ds(r, 8), :] = acc * inv

        def wo_task(t):
            r = t * TM
            lhs = _cat([o_v[c, pl.ds(r, TM), :].astype(BF16) for c in range(NC)], 1)
            rhs = _cat([_bf(wop[c]) for c in range(NC)], 1)
            y = jnp.dot(lhs, rhs, preferred_element_type=F32)
            for c in range(NC):
                att_v[c, pl.ds(r, TM), :] = y[:, c * 128:(c + 1) * 128]
            yield

        def ln2_task(r):
            att = _cat([att_v[c, pl.ds(r, 16), :] for c in range(NC)], 1)
            h = x_v[pl.ds(r, 16), :].astype(F32) + att
            m = jnp.sum(h, axis=-1, keepdims=True) * (1.0 / D)
            yield
            hc = h - m
            v = jnp.sum(hc * hc, axis=-1, keepdims=True) * (1.0 / D)
            yield
            hn = hc * lax.rsqrt(v + EPS)
            wr = wr_ref[...].astype(F32).reshape(1, D)
            rr = jnp.sum(hn * wr, axis=-1, keepdims=True)
            hn_v[pl.ds(r, 16), :] = hn.astype(BF16)
            out_v[pl.ds(r, 16), :] = (h + hn).astype(BF16)
            yield
            for g in range(2):
                rg = jnp.broadcast_to(rr[8 * g:8 * g + 8], (8, 128))
                idx = (r + 8 * g + lax.broadcasted_iota(I32, (8, 128), 0)).astype(F32)
                bv = best_v[0]
                better = rg > bv
                best_v[0] = jnp.where(better, rg, bv)
                best_v[1] = jnp.where(better, idx, best_v[1])

        def call_task(f):
            f()
            yield

        prep_w(1)
        prep_w(2)
        prep_w(0)
        x_copy(0).wait()
        run_interleaved([(j, ln1_task(16 * j), 0) for j in range(NJ)])
        for step in range(1, T + 3):
            t1, ta, tb, tc = step, step - 1, step - 2, step - 3
            if step == 2:
                for d in f_copies():
                    d.start()
                prep_wo()
            items = []
            if t1 < T:
                x_copy(t1).wait()
                items += [(2 * j, ln1_task(t1 * TM + 16 * j), order[0]) for j in range(NJ)]
            if 0 <= tc < T:
                items += [(0, wo_task(tc), order[1])]
                nt = NG - ln2_off - 3
                items += [(ln2_off + (j * nt) // NJ, ln2_task(tc * TM + 16 * j), order[4]) for j in range(NJ)]
            if 0 <= ta < T:
                items += [(mm_off + (n * (NG - mm_off)) // NCH, qkv_task(ta, n), order[2]) for n in range(NCH)]
            if 0 <= tb < T:
                items += [(g, attn_task(tb * TM + 8 * g), order[3]) for g in range(NG)]
            run_interleaved(items)
            if 0 <= tc < T:
                o_copy(tc).start()

        bv = best_v[0]
        bi = best_v[1]
        mx = jnp.max(bv, axis=0, keepdims=True)
        idxf = jnp.min(jnp.where(bv == mx, bi, 1e9), axis=0, keepdims=True)
        idxv = idxf.astype(I32)
        idx = idxv[0, 0]
        base = pl.multiple_of((idx // 16) * 16, 16)
        rows = lax.broadcasted_iota(I32, (16, D), 0)
        sel = rows == (idx - base)
        xs = jnp.where(sel, hn_v[pl.ds(base, 16), :].astype(F32), 0.0).astype(BF16)
        for d in f_copies():
            d.wait()
        g = jnp.dot(xs, wg_v[...], preferred_element_type=F32)
        u = jnp.dot(xs, wu_v[...], preferred_element_type=F32)
        a = (g * jax.nn.sigmoid(g) * u).astype(BF16)
        y = jnp.dot(a, wd_v[...], preferred_element_type=F32)
        gate = jax.nn.sigmoid(mx[:, 0:1])
        cur = out_v[pl.ds(base, 16), :].astype(F32)
        patch_v[...] = jnp.where(sel, cur + y * gate, cur).astype(BF16)
        for t in range(T):
            o_copy(t).wait()
        pc = pltpu.make_async_copy(patch_v, out_hbm.at[pl.ds(base, 16), :], sem_p)
        pc.start()
        pc.wait()

    def fn(A_x, A_wqkv, A_wo, B_x, B_w_r, B_w_gate, B_w_up, B_w_down):
        del B_x
        x2 = A_x.reshape(S, D)
        anyspec = pl.BlockSpec(memory_space=pl.ANY)
        out = pl.pallas_call(
            kern,
            out_shape=jax.ShapeDtypeStruct((S, D), BF16),
            in_specs=[anyspec, anyspec, anyspec, pl.BlockSpec(memory_space=pltpu.VMEM), anyspec, anyspec, anyspec],
            out_specs=anyspec,
            scratch_shapes=[
                pltpu.VMEM((S, D), BF16),
                pltpu.VMEM((3, D, D), BF16),
                pltpu.VMEM((D, D), BF16),
                pltpu.VMEM((4 * NC, 320, 128), I32),
                pltpu.VMEM((NC, 960, 128), I32),
                pltpu.VMEM((NC, 320, 128), I32),
                pltpu.VMEM((NC, S // 2, 128), I32),
                pltpu.VMEM((NC, S, 128), F32),
                pltpu.VMEM((NC, S + HALO, 128), F32),
                pltpu.VMEM((NC, S + HALO, 128), F32),
                pltpu.VMEM((NC, S, 128), F32),
                pltpu.VMEM((NC, S, 128), F32),
                pltpu.VMEM((S, D), BF16),
                pltpu.VMEM((S, D), BF16),
                pltpu.VMEM((D, F), BF16),
                pltpu.VMEM((D, F), BF16),
                pltpu.VMEM((F, D), BF16),
                pltpu.VMEM((2, 8, 128), F32),
                pltpu.VMEM((16, D), BF16),
                pltpu.SemaphoreType.DMA((T,)),
                pltpu.SemaphoreType.DMA((4,)),
                pltpu.SemaphoreType.DMA((3,)),
                pltpu.SemaphoreType.DMA((T,)),
                pltpu.SemaphoreType.DMA(()),
            ],
            compiler_params=pltpu.CompilerParams(vmem_limit_bytes=110 * 2 ** 20),
        )(x2, A_wqkv, A_wo, B_w_r, B_w_gate, B_w_up, B_w_down)
        return out.reshape(1, S, D)

    return fn


_IMPL = {}


@jax.jit
def pallas_sequential_preLN__sliding_local_dilated__moe_arch_mod__prompt_kernel(
    A_x: jax.Array,
    A_wqkv: jax.Array,
    A_wo: jax.Array,
    B_x: jax.Array,
    B_w_r: jax.Array,
    B_w_gate: jax.Array,
    B_w_up: jax.Array,
    B_w_down: jax.Array,
):
    return make_kernel()(A_x, A_wqkv, A_wo, B_x, B_w_r, B_w_gate, B_w_up, B_w_down)
```

```python
import contextlib
import jax
import jax.numpy as jnp
import numpy as np
from jax import lax
from jax.experimental import pallas as pl
from jax.experimental.pallas import tpu as pltpu

S, D, F = 2048, 640, 1536
H, DH, W, DIL = 32, 20, 8, 2
NC = D // 128
HALO = 16
F32 = jnp.float32
BF16 = jnp.bfloat16
I32 = jnp.int32
LOG2E = 1.4426950408889634
QSCALE = float(DH ** -0.5) * LOG2E
NEG = -1e9 * LOG2E
EPS = 1e-5


def _cat(xs, axis):
    return xs[0] if len(xs) == 1 else jnp.concatenate(xs, axis=axis)


def _regroup(src_ref, c, dp):
    a = src_ref[c, pl.ds(dp, 16, stride=20), :]
    b = src_ref[c, pl.ds(10 + dp, 16, stride=20), :]
    lo = jnp.bitwise_or(jnp.bitwise_and(a, 0xFFFF), jnp.left_shift(b, 16))
    hi = jnp.bitwise_or(lax.shift_right_logical(a, 16), jnp.bitwise_and(b, -65536))
    return lo, hi


def _bf(x):
    return pltpu.bitcast(x, BF16)


def _i32(x):
    return pltpu.bitcast(x, I32)


def run_interleaved(streams, rev=False):
    active = []
    pending = sorted(streams, key=lambda t: t[0])
    tick = 0
    while pending or active:
        while pending and pending[0][0] <= tick:
            active.append(pending.pop(0))
        active.sort(key=lambda t: (t[2], -t[0] if rev else t[0]))
        nxt = []
        for item in active:
            try:
                next(item[1])
                nxt.append(item)
            except StopIteration:
                pass
        active = nxt
        tick += 1


def default_plan():
    P = [{'ln1': (0, 128), 'wait': ['x0']},
 {'prep': ['k'], 'wait': ['wk']},
 {'ln1': (128, 384), 'mm': [('qkv', 1, 0, 128)], 'wait': ['x1']},
 {'mm': [('qkv', 1, 128, 256)], 'prep': ['v'], 'wait': ['wv']},
 {'mm': [('qkv', 2, 0, 384)], 'prep': ['q'], 'wait': ['wq']},
 {'att': (0, 128), 'ln1': (384, 640), 'mm': [('qkv', 0, 0, 128), ('qkv', 0, 128, 256)], 'wait': ['x2']},
 {'att': (128, 384), 'ln1': (640, 896), 'mm': [('qkv3', 384, 256)], 'prep': ['o'], 'start': ['ffn'], 'wait': ['x3', 'wo', 'wr']},
 {'att': (384, 640), 'ln1': (896, 1152), 'mm': [('qkv3', 640, 256), ('wo', 0, 384)], 'wait': ['x4']},
 {'att': (640, 896), 'ln1': (1152, 1408), 'ln2': [(0, 384)], 'mm': [('qkv3', 896, 256), ('wo', 384, 256)], 'wait': ['x5']},
 {'att': (896, 1152), 'ln1': (1408, 1664), 'ln2': [(384, 640)], 'mm': [('qkv3', 1152, 256), ('wo', 640, 256)], 'wait': ['x6']},
 {'att': (1152, 1408), 'ln1': (1664, 1920), 'ln2': [(640, 896)], 'mm': [('qkv3', 1408, 256), ('wo', 896, 256)], 'ostart': (0, 640), 'wait': ['x7']},
 {'att': (1408, 1664),
  'ln1': (1920, 2048),
  'ln2': [(896, 1152)],
  'mm': [('qkv3', 1664, 256), ('wo', 1152, 256)],
  'ostart': (640, 896),
  'wait': ['x8']},
 {'att': (1664, 1920), 'ln2': [(1152, 1408)], 'mm': [('qkv3', 1920, 128), ('wo', 1408, 256)], 'ostart': (896, 1152), 'wait': ['wg']},
 {'att': (1920, 2048),
  'ln2': [(1408, 1664), (1664, 1920), (1920, 2048)],
  'ln2batch': 4,
  'mm': [('wo', 1664, 256), ('wo', 1920, 128)],
  'ostart': (1152, 1408),
  'wait': ['wu']},
 {'ostart': (1408, 2048)}]
    xg = [(0, 128), (128, 384), (384, 640), (640, 896), (896, 1152), (1152, 1408), (1408, 1664), (1664, 1920), (1920, 2048)]
    order = ['x0', 'wk', 'x1', 'wv', 'wq', 'x2', 'wo', 'wr', 'x3', 'x4', 'x5', 'x6', 'x7', 'x8']
    return P, xg, order


def make_kernel(plan=None, rev=False, dbg=None, flags=None, gates=None, gfrac=(0.25, 0.5, 0.75), abl=''):
    P, xgroups, dma_order = default_plan()
    ogroups = [p['ostart'] for p in P if 'ostart' in p]
    NO = len(ogroups)

    def kern(z_ref, x_hbm, wqkv_hbm, wo_hbm, wr_hbm, wg_hbm, wu_hbm, wd_hbm, out_hbm,
             x_v, wraw, woraw, t32, wtp, wop, xn_v, q_v, k_v, v_v, att_v, out_v, o_v,
             wg_v, wu_v, wd_v, wr_v, patch_v, sem_x, sem_w, sem_f, sem_o, sem_p):
        scope = (lambda n: jax.named_scope(n)) if dbg == 'scopes' else (lambda n: contextlib.nullcontext())

        def dma(name):
            if name[0] == 'x':
                gi = int(name[1:])
                a, b = xgroups[gi]
                return pltpu.make_async_copy(x_hbm.at[pl.ds(a, b - a), :], x_v.at[pl.ds(a, b - a), :], sem_x.at[gi])
            if name in ('wq', 'wk', 'wv'):
                p = ('wq', 'wk', 'wv').index(name)
                return pltpu.make_async_copy(wqkv_hbm.at[:, pl.ds(p * D, D)], wraw.at[p], sem_w.at[p])
            if name == 'wo':
                return pltpu.make_async_copy(wo_hbm, woraw, sem_w.at[3])
            if name == 'wr':
                return pltpu.make_async_copy(wr_hbm, wr_v, sem_w.at[4])
            if name in ('wg', 'wu', 'wd'):
                return f_copy(('wg', 'wu', 'wd').index(name))
            if name[0] == 'o':
                return o_copy(int(name[1:]))
            raise KeyError(name)

        def f_copy(i):
            return pltpu.make_async_copy((wg_hbm, wu_hbm, wd_hbm)[i], (wg_v, wu_v, wd_v)[i], sem_f.at[i])

        def o_copy(i):
            a, b = ogroups[i]
            if 'c' in abl:
                return [pltpu.make_async_copy(out_v.at[c, pl.ds(a, b - a), :], out_hbm.at[pl.ds(a, b - a), pl.ds(c * 128, 128)], sem_o.at[i * NC + c]) for c in range(NC)]
            return [pltpu.make_async_copy(out_v.at[pl.ds(a, b - a), :], out_hbm.at[pl.ds(a, b - a), :], sem_o.at[i * NC])]

        zdyn = pl.multiple_of(z_ref[0], 16)
        for name in dma_order:
            dma(name).start()

        zeros = jnp.zeros((HALO, 128), F32)
        for c in range(NC):
            k_v[c, pl.ds(0, HALO), :] = zeros
            v_v[c, pl.ds(0, HALO), :] = zeros
        q_v[0, pl.ds(S, 16), :] = zeros
        best = [jnp.full((8, 128), -jnp.inf, F32), jnp.zeros((8, 128), F32)]

        def prep_w(p):
            for kt in range(NC):
                for ft in range(NC):
                    tile = wraw[p, pl.ds(kt * 128, 128), pl.ds(ft * 128, 128)]
                    t32[p * NC + kt, pl.ds(64 * ft, 64), :] = _i32(tile.T)
            for kt in range(NC):
                for dp in range(10):
                    lo, hi = _regroup(t32, p * NC + kt, dp)
                    wtp[kt, pl.ds(p * 320 + 32 * dp, 16), :] = lo
                    wtp[kt, pl.ds(p * 320 + 32 * dp + 16, 16), :] = hi

        def prep_wo():
            for c in range(NC):
                t32[3 * NC + c] = _i32(woraw[:, pl.ds(c * 128, 128)])
            for c in range(NC):
                for dp in range(10):
                    lo, hi = _regroup(t32, 3 * NC + c, dp)
                    wop[c, pl.ds(32 * dp, 16), :] = lo
                    wop[c, pl.ds(32 * dp + 16, 16), :] = hi

        def load_bf(ref, c, r, n):
            return _bf(ref[c, pl.ds(r // 2, n // 2), :])

        def gate(which, n):
            if which == 'k':
                return k_v[0, pl.ds(zdyn, n), :]
            if which == 'v':
                return v_v[0, pl.ds(zdyn, n), :]
            return q_v[0, pl.ds(pl.multiple_of(zdyn + S, 16), n), :]

        def ln1_task(r, gt=None):
            xf = x_v[pl.ds(r, 16), :].astype(F32)
            if gt:
                g = gate(gt, 16)
                xf = _cat([xf[:, c * 128:(c + 1) * 128] + g for c in range(NC)], 1)
            m = jnp.sum(xf, axis=-1, keepdims=True) * (1.0 / D)
            yield
            xc = xf - m
            v = jnp.sum(xc * xc, axis=-1, keepdims=True) * (1.0 / D)
            yield
            xn = (xc * lax.rsqrt(v + EPS)).astype(BF16)
            for c in range(NC):
                xn_v[c, pl.ds(r // 2, 8), :] = _i32(xn[:, c * 128:(c + 1) * 128])

        def qkv_task(p, r, n):
            lhs = _cat([load_bf(xn_v, c, r, n) for c in range(NC)], 1)
            rhs = _cat([load_bf(wtp, c, p * D, D) for c in range(NC)], 1)
            y = lax.dot_general(lhs, rhs, (((1,), (1,)), ((), ())), preferred_element_type=F32)
            for c in range(NC):
                yc = y[:, c * 128:(c + 1) * 128]
                if p == 0:
                    q_v[c, pl.ds(r, n), :] = yc * QSCALE
                elif p == 1:
                    k_v[c, pl.ds(HALO + r, n), :] = yc
                else:
                    v_v[c, pl.ds(HALO + r, n), :] = yc
            yield

        def attn_task(r, gt=None):
            q = [q_v[c, pl.ds(r, 8), :] for c in range(NC)]
            if gt:
                g = gate(gt, 8)
                q = [a + g for a in q]
            s = []
            for w in range(W):
                acc = None
                for c in range(NC):
                    pr = q[c] * k_v[c, pl.ds(HALO + r - DIL * w, 8), :]
                    acc = pr if acc is None else acc + pr
                s.append(acc)
            rr = [pltpu.roll(a, 64, 1) for a in s] if 'r' not in abl else s
            yield
            s = [a + b for a, b in zip(s, rr)]
            rr = [pltpu.roll(a, 32, 1) for a in s] if 'r' not in abl else s
            yield
            s = [a + b for a, b in zip(s, rr)]
            for w in range(W):
                if r < DIL * w:
                    rows = r + lax.broadcasted_iota(I32, (8, 128), 0)
                    s[w] = jnp.where(rows >= DIL * w, s[w], NEG)
            m = s[0]
            for w in range(1, W):
                m = jnp.maximum(m, s[w])
            p = [jnp.exp2(s[w] - m) for w in range(W)]
            l = p[0]
            for w in range(1, W):
                l = l + p[w]
            if True:
                y0 = pl.reciprocal(l, approx=True)
                inv = y0 * (2.0 - l * y0)
            else:
                inv = 1.0 / l
            for c in range(NC):
                acc = None
                for w in range(W):
                    pr = p[w] * v_v[c, pl.ds(HALO + r - DIL * w, 8), :]
                    acc = pr if acc is None else acc + pr
                o_v[c, pl.ds(r, 8), :] = acc * inv

        def wo_task(r, n):
            lhs = _cat([o_v[c, pl.ds(r, n), :].astype(BF16) for c in range(NC)], 1)
            rhs = _cat([load_bf(wop, c, 0, D) for c in range(NC)], 1)
            y = jnp.dot(lhs, rhs, preferred_element_type=F32)
            for c in range(NC):
                att_v[c, pl.ds(r, n), :] = y[:, c * 128:(c + 1) * 128]
            yield

        def ln2_task(r, gt=None):
            att = [att_v[c, pl.ds(r, 16), :] for c in range(NC)]
            if gt:
                g = gate(gt, 16)
                att = [a + g for a in att]
            att = _cat(att, 1)
            h = x_v[pl.ds(r, 16), :].astype(F32) + att
            m = jnp.sum(h, axis=-1, keepdims=True) * (1.0 / D)
            yield
            hc = h - m
            v = jnp.sum(hc * hc, axis=-1, keepdims=True) * (1.0 / D)
            yield
            hn = hc * lax.rsqrt(v + EPS)
            wr = wr_v[...].astype(F32).reshape(1, D)
            rr = jnp.sum(hn * wr, axis=-1, keepdims=True)
            ob = (h + hn).astype(BF16)
            if 'c' in abl:
                for c in range(NC):
                    out_v[c, pl.ds(r, 16), :] = ob[:, c * 128:(c + 1) * 128]
            else:
                out_v[pl.ds(r, 16), :] = ob
            yield
            for g in range(2 if 'b' not in abl else 0):
                rg = jnp.broadcast_to(rr[8 * g:8 * g + 8], (8, 128))
                idx = (r + 8 * g + lax.broadcasted_iota(I32, (8, 128), 0)).astype(F32)
                bv, bi = best
                better = rg > bv
                best[0] = jnp.where(better, rg, bv)
                best[1] = jnp.where(better, idx, bi)

        def call_task(f, *a):
            f(*a)
            yield

        oi = 0
        for ri, reg in enumerate(P):
            for name in reg.get('wait', []):
                dma(name).wait()
            if 'ffn' in reg.get('start', []):
                for i in range(3):
                    f_copy(i).start()
            if 'ostart' in reg:
                for d in o_copy(oi):
                    d.start()
                oi += 1
            mm = []
            for job in reg.get('mm', []):
                if job[0] == 'qkv3':
                    mm += [('qkv', p, job[1], job[2]) for p in (1, 2, 0)]
                else:
                    mm.append(job)
            NT = max(1, sum(j[-1] for j in mm) // 32)
            ln2 = reg.get('ln2', [])
            NT = max([NT] + [(reg[k][1] - reg[k][0]) // 8 for k in ('ln1', 'att') if k in reg] + [(b - a) // 8 for a, b in ln2])
            parts = [j[1] for j in mm if j[0] == 'qkv']
            gated = gates and len(parts) == 3 and len(set(parts)) == 3

            def gsel(frac, kind):
                if not gated or kind not in gates:
                    return None
                g = None
                for f, nm in zip(gfrac, 'kvq'):
                    if frac >= f:
                        g = nm
                return g
            items = []
            for pn in reg.get('prep', []):
                items.append((0, call_task(prep_wo) if pn == 'o' else call_task(prep_w, 'qkv'.index(pn) if pn == 'q' else {'k': 1, 'v': 2}[pn]), 9))
            if 'ln1' in reg and not ('1' in abl and ri > 5):
                a, b = reg['ln1']
                nj = (b - a) // 16
                items += [((j * NT) // nj, ln1_task(a + 16 * j, gsel(j / nj, '1')), 0) for j in range(nj)]
            tot = sum(j[-1] for j in mm)
            acc = 0
            for job in mm:
                pos = (acc * NT) // tot
                acc += job[-1]
                if job[0] == 'qkv':
                    items.append((pos, qkv_task(*job[1:]), 1))
                else:
                    if 'att' in reg and job[1] + job[2] > reg['att'][0]:
                        pos = NT + 2
                    items.append((pos, wo_task(*job[1:]), 1))
            nl = len(ln2)
            if '2' in abl:
                ln2 = []
            for li, (a, b) in enumerate(ln2):
                nj = (b - a) // 16
                bt = reg.get('ln2batch', 1)
                items += [(li * NT + ((j // bt) * bt * NT) // nj + 1, ln2_task(a + 16 * j, gsel(j / nj, '2')), 4) for j in range(nj)]
            if 'att' in reg and 'a' not in abl:
                a, b = reg['att']
                ng = (b - a) // 8
                items += [((g * NT) // ng, attn_task(a + 8 * g, gsel(g / ng, 'a')), 3) for g in range(ng)]
            with scope(f'reg{ri:02d}'):
                run_interleaved(items, rev)

        with scope('tail'):
            bv, bi = best
            mx = jnp.max(bv, axis=0, keepdims=True)
            idxf = jnp.min(jnp.where(bv == mx, bi, 1e9), axis=0, keepdims=True)
            idxv = idxf.astype(I32)
            idx = idxv[0, 0]
            base = pl.multiple_of((idx // 16) * 16, 16)
            rows = lax.broadcasted_iota(I32, (16, D), 0)
            sel = rows == (idx - base)
            hb = x_v[pl.ds(base, 16), :].astype(F32) + _cat([att_v[c, pl.ds(base, 16), :] for c in range(NC)], 1)
            hcb = hb - jnp.sum(hb, axis=-1, keepdims=True) * (1.0 / D)
            hnb = hcb * lax.rsqrt(jnp.sum(hcb * hcb, axis=-1, keepdims=True) * (1.0 / D) + EPS)
            xs = jnp.where(sel, hnb, 0.0).astype(BF16)
            waited = [n for p in P for n in p.get('wait', [])]
            for n in ('wg', 'wu', 'wd'):
                if n not in waited:
                    dma(n).wait()
            g = jnp.dot(xs, wg_v[...], preferred_element_type=F32)
            u = jnp.dot(xs, wu_v[...], preferred_element_type=F32)
            a = (g * jax.nn.sigmoid(g) * u).astype(BF16)
            y = jnp.dot(a, wd_v[...], preferred_element_type=F32)
            gate = jax.nn.sigmoid(mx[:, 0:1])
            cur = hb + hnb
            patch_v[...] = jnp.where(sel, cur + y * gate, cur).astype(BF16)
        with scope('tail_dma'):
            for i in range(NO):
                if f'o{i}' not in waited:
                    for d in o_copy(i):
                        d.wait()
            pc = pltpu.make_async_copy(patch_v, out_hbm.at[pl.ds(base, 16), :], sem_p)
            pc.start()
            pc.wait()

    def fn(A_x, A_wqkv, A_wo, B_x, B_w_r, B_w_gate, B_w_up, B_w_down):
        del B_x
        x2 = A_x.reshape(S, D)
        anyspec = pl.BlockSpec(memory_space=pl.ANY)
        out = pl.pallas_call(
            kern,
            out_shape=jax.ShapeDtypeStruct((S, D), BF16),
            in_specs=[pl.BlockSpec(memory_space=pltpu.SMEM)] + [anyspec] * 7,
            out_specs=anyspec,
            scratch_shapes=[
                pltpu.VMEM((S, D), BF16),
                pltpu.VMEM((3, D, D), BF16),
                pltpu.VMEM((D, D), BF16),
                pltpu.VMEM((4 * NC, 320, 128), I32),
                pltpu.VMEM((NC, 960, 128), I32),
                pltpu.VMEM((NC, 320, 128), I32),
                pltpu.VMEM((NC, S // 2, 128), I32),
                pltpu.VMEM((NC, S + 16, 128), F32),
                pltpu.VMEM((NC, S + HALO, 128), F32),
                pltpu.VMEM((NC, S + HALO, 128), F32),
                pltpu.VMEM((NC, S, 128), F32),
                pltpu.VMEM((NC, S, 128), BF16) if 'c' in abl else pltpu.VMEM((S, D), BF16),
                pltpu.VMEM((NC, S, 128), F32),
                pltpu.VMEM((D, F), BF16),
                pltpu.VMEM((D, F), BF16),
                pltpu.VMEM((F, D), BF16),
                pltpu.VMEM((D,), BF16),
                pltpu.VMEM((16, D), BF16),
                pltpu.SemaphoreType.DMA((len(xgroups),)),
                pltpu.SemaphoreType.DMA((5,)),
                pltpu.SemaphoreType.DMA((3,)),
                pltpu.SemaphoreType.DMA((NO * NC,)),
                pltpu.SemaphoreType.DMA(()),
            ],
            compiler_params=pltpu.CompilerParams(vmem_limit_bytes=110 * 2 ** 20, flags=flags),
        )(np.zeros((1,), np.int32), x2, A_wqkv, A_wo, B_w_r, B_w_gate, B_w_up, B_w_down)
        return out.reshape(1, S, D)

    return fn


@jax.jit
def pallas_sequential_preLN__sliding_local_dilated__moe_arch_mod__prompt_kernel(
    A_x: jax.Array,
    A_wqkv: jax.Array,
    A_wo: jax.Array,
    B_x: jax.Array,
    B_w_r: jax.Array,
    B_w_gate: jax.Array,
    B_w_up: jax.Array,
    B_w_down: jax.Array,
):
    return make_kernel(rev=True)(A_x, A_wqkv, A_wo, B_x, B_w_r, B_w_gate, B_w_up, B_w_down)
```

```python
import contextlib
import jax
import jax.numpy as jnp
import numpy as np
from jax import lax
from jax.experimental import pallas as pl
from jax.experimental.pallas import tpu as pltpu

S, D, F = 2048, 640, 1536
H, DH, W, DIL = 32, 20, 8, 2
NC = D // 128
HALO = 16
F32 = jnp.float32
BF16 = jnp.bfloat16
I32 = jnp.int32
LOG2E = 1.4426950408889634
QSCALE = float(DH ** -0.5) * LOG2E
NEG = -1e9 * LOG2E
EPS = 1e-5


def _cat(xs, axis):
    return xs[0] if len(xs) == 1 else jnp.concatenate(xs, axis=axis)


def _regroup(src_ref, c, dp):
    a = src_ref[c, pl.ds(dp, 16, stride=20), :]
    b = src_ref[c, pl.ds(10 + dp, 16, stride=20), :]
    lo = jnp.bitwise_or(jnp.bitwise_and(a, 0xFFFF), jnp.left_shift(b, 16))
    hi = jnp.bitwise_or(lax.shift_right_logical(a, 16), jnp.bitwise_and(b, -65536))
    return lo, hi


def _bf(x):
    return pltpu.bitcast(x, BF16)


def _i32(x):
    return pltpu.bitcast(x, I32)


def run_interleaved(streams, rev=False):
    active = []
    pending = sorted(streams, key=lambda t: t[0])
    tick = 0
    while pending or active:
        while pending and pending[0][0] <= tick:
            active.append(pending.pop(0))
        active.sort(key=lambda t: (t[2], -t[0] if rev else t[0]))
        nxt = []
        for item in active:
            try:
                next(item[1])
                nxt.append(item)
            except StopIteration:
                pass
        active = nxt
        tick += 1


def default_plan():
    P = [{'ln1': (0, 128), 'wait': ['x0']},
 {'prep': ['k'], 'wait': ['wk']},
 {'ln1': (128, 384), 'mm': [('qkv', 1, 0, 128)], 'wait': ['x1']},
 {'mm': [('qkv', 1, 128, 256)], 'prep': ['v'], 'wait': ['wv']},
 {'mm': [('qkv', 2, 0, 384)], 'prep': ['q'], 'wait': ['wq', 'x2']},
 {'att': (0, 128), 'ln1': (384, 640), 'mm': [('qkv', 0, 0, 128), ('qkv', 0, 128, 256)], 'wait': []},
 {'att': (128, 384), 'ln1': (640, 896), 'mm': [('qkv3', 384, 256)], 'prep': ['o'], 'start': ['ffn'], 'wait': ['x3', 'wo', 'wr']},
 {'att': (384, 640), 'ln1': (896, 1152), 'mm': [('qkv3', 640, 256), ('wo', 0, 384)], 'wait': ['x4']},
 {'att': (640, 896), 'ln1': (1152, 1408), 'ln2': [(0, 384)], 'mm': [('qkv3', 896, 256), ('wo', 384, 256)], 'wait': ['x5']},
 {'att': (896, 1152), 'ln1': (1408, 1664), 'ln2': [(384, 640)], 'mm': [('qkv3', 1152, 256), ('wo', 640, 256)], 'wait': ['x6']},
 {'att': (1152, 1408), 'ln1': (1664, 1920), 'ln2': [(640, 896)], 'mm': [('qkv3', 1408, 256), ('wo', 896, 256)], 'ostart': (0, 640), 'wait': ['x7']},
 {'att': (1408, 1664),
  'ln1': (1920, 2048),
  'ln2': [(896, 1152)],
  'mm': [('qkv3', 1664, 256), ('wo', 1152, 256)],
  'ostart': (640, 896),
  'wait': ['x8']},
 {'att': (1664, 1920), 'ln2': [(1152, 1408)], 'mm': [('qkv3', 1920, 128), ('wo', 1408, 256)], 'ostart': (896, 1152), 'wait': ['wg']},
 {'att': (1920, 2048),
  'ln2': [(1408, 1664), (1664, 1920), (1920, 2048)],
  'ln2batch': 4,
  'mm': [('wo', 1664, 256), ('wo', 1920, 128)],
  'ostart': (1152, 1408),
  'wait': ['wu']},
 {'ostart': (1408, 2048)}]
    xg = [(0, 128), (128, 384), (384, 640), (640, 896), (896, 1152), (1152, 1408), (1408, 1664), (1664, 1920), (1920, 2048)]
    order = ['x0', 'wk', 'x1', 'wv', 'x2', 'wq', 'wo', 'wr', 'x3', 'x4', 'x5', 'x6', 'x7', 'x8']
    return P, xg, order


def make_kernel(plan=None, rev=False, dbg=None, flags=None, gates=None, gfrac=(0.25, 0.5, 0.75), abl=''):
    P, xgroups, dma_order = default_plan()
    ogroups = [p['ostart'] for p in P if 'ostart' in p]
    NO = len(ogroups)

    def kern(z_ref, x_hbm, wqkv_hbm, wo_hbm, wr_hbm, wg_hbm, wu_hbm, wd_hbm, out_hbm,
             x_v, wraw, woraw, t32, wtp, wop, xn_v, q_v, k_v, v_v, att_v, out_v, o_v,
             wg_v, wu_v, wd_v, wr_v, patch_v, sem_x, sem_w, sem_f, sem_o, sem_p):
        scope = (lambda n: jax.named_scope(n)) if dbg == 'scopes' else (lambda n: contextlib.nullcontext())

        def dma(name):
            if name[0] == 'x':
                gi = int(name[1:])
                a, b = xgroups[gi]
                return pltpu.make_async_copy(x_hbm.at[pl.ds(a, b - a), :], x_v.at[pl.ds(a, b - a), :], sem_x.at[gi])
            if name in ('wq', 'wk', 'wv'):
                p = ('wq', 'wk', 'wv').index(name)
                return pltpu.make_async_copy(wqkv_hbm.at[:, pl.ds(p * D, D)], wraw.at[p], sem_w.at[p])
            if name == 'wo':
                return pltpu.make_async_copy(wo_hbm, woraw, sem_w.at[3])
            if name == 'wr':
                return pltpu.make_async_copy(wr_hbm, wr_v, sem_w.at[4])
            if name in ('wg', 'wu', 'wd'):
                return f_copy(('wg', 'wu', 'wd').index(name))
            if name[0] == 'o':
                return o_copy(int(name[1:]))
            raise KeyError(name)

        def f_copy(i):
            return pltpu.make_async_copy((wg_hbm, wu_hbm, wd_hbm)[i], (wg_v, wu_v, wd_v)[i], sem_f.at[i])

        def o_copy(i):
            a, b = ogroups[i]
            if 'c' in abl:
                return [pltpu.make_async_copy(out_v.at[c, pl.ds(a, b - a), :], out_hbm.at[pl.ds(a, b - a), pl.ds(c * 128, 128)], sem_o.at[i * NC + c]) for c in range(NC)]
            return [pltpu.make_async_copy(out_v.at[pl.ds(a, b - a), :], out_hbm.at[pl.ds(a, b - a), :], sem_o.at[i * NC])]

        zdyn = pl.multiple_of(z_ref[0], 16)
        for name in dma_order:
            dma(name).start()

        zeros = jnp.zeros((HALO, 128), F32)
        for c in range(NC):
            k_v[c, pl.ds(0, HALO), :] = zeros
            v_v[c, pl.ds(0, HALO), :] = zeros
        q_v[0, pl.ds(S, 16), :] = zeros
        best = [jnp.full((8, 128), -jnp.inf, F32), jnp.zeros((8, 128), F32)]

        def prep_w(p):
            for kt in range(NC):
                for ft in range(NC):
                    tile = wraw[p, pl.ds(kt * 128, 128), pl.ds(ft * 128, 128)]
                    t32[p * NC + kt, pl.ds(64 * ft, 64), :] = _i32(tile.T)
            for kt in range(NC):
                for dp in range(10):
                    lo, hi = _regroup(t32, p * NC + kt, dp)
                    wtp[kt, pl.ds(p * 320 + 32 * dp, 16), :] = lo
                    wtp[kt, pl.ds(p * 320 + 32 * dp + 16, 16), :] = hi

        def prep_wo():
            for c in range(NC):
                t32[3 * NC + c] = _i32(woraw[:, pl.ds(c * 128, 128)])
            for c in range(NC):
                for dp in range(10):
                    lo, hi = _regroup(t32, 3 * NC + c, dp)
                    wop[c, pl.ds(32 * dp, 16), :] = lo
                    wop[c, pl.ds(32 * dp + 16, 16), :] = hi

        def load_bf(ref, c, r, n):
            return _bf(ref[c, pl.ds(r // 2, n // 2), :])

        done = {k: set() for k in ('x', 'xn', 0, 1, 2, 'o', 'att', 'out')}

        def need(k, a, b):
            assert all(r in done[k] for r in range(max(a, 0), b)), (k, a, b)

        def mark(k, a, b):
            done[k].update(range(a, b))

        def gate(which, n):
            if which == 'k':
                return k_v[0, pl.ds(zdyn, n), :]
            if which == 'v':
                return v_v[0, pl.ds(zdyn, n), :]
            return q_v[0, pl.ds(pl.multiple_of(zdyn + S, 16), n), :]

        def ln1_task(r, gt=None):
            need('x', r, r + 16)
            xf = x_v[pl.ds(r, 16), :].astype(F32)
            if gt:
                g = gate(gt, 16)
                xf = _cat([xf[:, c * 128:(c + 1) * 128] + g for c in range(NC)], 1)
            m = jnp.sum(xf, axis=-1, keepdims=True) * (1.0 / D)
            yield
            xc = xf - m
            v = jnp.sum(xc * xc, axis=-1, keepdims=True) * (1.0 / D)
            yield
            xn = (xc * lax.rsqrt(v + EPS)).astype(BF16)
            for c in range(NC):
                xn_v[c, pl.ds(r // 2, 8), :] = _i32(xn[:, c * 128:(c + 1) * 128])
            mark('xn', r, r + 16)

        def qkv_task(p, r, n):
            need('xn', r, r + n)
            mark(p, r, r + n)
            lhs = _cat([load_bf(xn_v, c, r, n) for c in range(NC)], 1)
            rhs = _cat([load_bf(wtp, c, p * D, D) for c in range(NC)], 1)
            y = lax.dot_general(lhs, rhs, (((1,), (1,)), ((), ())), preferred_element_type=F32)
            for c in range(NC):
                yc = y[:, c * 128:(c + 1) * 128]
                if p == 0:
                    q_v[c, pl.ds(r, n), :] = yc * QSCALE
                elif p == 1:
                    k_v[c, pl.ds(HALO + r, n), :] = yc
                else:
                    v_v[c, pl.ds(HALO + r, n), :] = yc
            yield

        def attn_task(r, gt=None):
            need(0, r, r + 8)
            need(1, r - 14, r + 8)
            need(2, r - 14, r + 8)
            q = [q_v[c, pl.ds(r, 8), :] for c in range(NC)]
            if gt:
                g = gate(gt, 8)
                q = [a + g for a in q]
            s = []
            for w in range(W):
                acc = None
                for c in range(NC):
                    pr = q[c] * k_v[c, pl.ds(HALO + r - DIL * w, 8), :]
                    acc = pr if acc is None else acc + pr
                s.append(acc)
            rr = [pltpu.roll(a, 64, 1) for a in s] if 'r' not in abl else s
            yield
            s = [a + b for a, b in zip(s, rr)]
            rr = [pltpu.roll(a, 32, 1) for a in s] if 'r' not in abl else s
            yield
            s = [a + b for a, b in zip(s, rr)]
            for w in range(W):
                if r < DIL * w:
                    rows = r + lax.broadcasted_iota(I32, (8, 128), 0)
                    s[w] = jnp.where(rows >= DIL * w, s[w], NEG)
            m = s[0]
            for w in range(1, W):
                m = jnp.maximum(m, s[w])
            p = [jnp.exp2(s[w] - m) for w in range(W)]
            l = p[0]
            for w in range(1, W):
                l = l + p[w]
            if True:
                y0 = pl.reciprocal(l, approx=True)
                inv = y0 * (2.0 - l * y0)
            else:
                inv = 1.0 / l
            for c in range(NC):
                acc = None
                for w in range(W):
                    pr = p[w] * v_v[c, pl.ds(HALO + r - DIL * w, 8), :]
                    acc = pr if acc is None else acc + pr
                o_v[c, pl.ds(r, 8), :] = acc * inv
            mark('o', r, r + 8)

        def wo_task(r, n):
            need('o', r, r + n)
            mark('att', r, r + n)
            lhs = _cat([o_v[c, pl.ds(r, n), :].astype(BF16) for c in range(NC)], 1)
            rhs = _cat([load_bf(wop, c, 0, D) for c in range(NC)], 1)
            y = jnp.dot(lhs, rhs, preferred_element_type=F32)
            for c in range(NC):
                att_v[c, pl.ds(r, n), :] = y[:, c * 128:(c + 1) * 128]
            yield

        def ln2_task(r, gt=None):
            need('att', r, r + 16)
            att = [att_v[c, pl.ds(r, 16), :] for c in range(NC)]
            if gt:
                g = gate(gt, 16)
                att = [a + g for a in att]
            att = _cat(att, 1)
            h = x_v[pl.ds(r, 16), :].astype(F32) + att
            m = jnp.sum(h, axis=-1, keepdims=True) * (1.0 / D)
            yield
            hc = h - m
            v = jnp.sum(hc * hc, axis=-1, keepdims=True) * (1.0 / D)
            yield
            hn = hc * lax.rsqrt(v + EPS)
            wr = wr_v[...].astype(F32).reshape(1, D)
            rr = jnp.sum(hn * wr, axis=-1, keepdims=True)
            ob = (h + hn).astype(BF16)
            if 'c' in abl:
                for c in range(NC):
                    out_v[c, pl.ds(r, 16), :] = ob[:, c * 128:(c + 1) * 128]
            else:
                out_v[pl.ds(r, 16), :] = ob
            mark('out', r, r + 16)
            yield
            for g in range(2 if 'b' not in abl else 0):
                rg = jnp.broadcast_to(rr[8 * g:8 * g + 8], (8, 128))
                idx = (r + 8 * g + lax.broadcasted_iota(I32, (8, 128), 0)).astype(F32)
                bv, bi = best
                better = rg > bv
                best[0] = jnp.where(better, rg, bv)
                best[1] = jnp.where(better, idx, bi)

        def call_task(f, *a):
            f(*a)
            yield

        oi = 0
        for ri, reg in enumerate(P):
            for name in reg.get('wait', []):
                dma(name).wait()
                if name[0] == 'x':
                    mark('x', *xgroups[int(name[1:])])
            if 'ffn' in reg.get('start', []):
                for i in range(3):
                    f_copy(i).start()
            if 'ostart' in reg:
                need('out', *reg['ostart'])
                for d in o_copy(oi):
                    d.start()
                oi += 1
            mm = []
            for job in reg.get('mm', []):
                if job[0] == 'qkv3':
                    mm += [('qkv', p, job[1], job[2]) for p in (1, 2, 0)]
                else:
                    mm.append(job)
            NT = max(1, sum(j[-1] for j in mm) // 32)
            ln2 = reg.get('ln2', [])
            NT = max([NT] + [(reg[k][1] - reg[k][0]) // 8 for k in ('ln1', 'att') if k in reg] + [(b - a) // 8 for a, b in ln2])
            parts = [j[1] for j in mm if j[0] == 'qkv']
            gated = gates and len(parts) == 3 and len(set(parts)) == 3

            def gsel(frac, kind):
                if not gated or kind not in gates:
                    return None
                g = None
                for f, nm in zip(gfrac, 'kvq'):
                    if frac >= f:
                        g = nm
                return g
            items = []
            for pn in reg.get('prep', []):
                items.append((0, call_task(prep_wo) if pn == 'o' else call_task(prep_w, 'qkv'.index(pn) if pn == 'q' else {'k': 1, 'v': 2}[pn]), 9))
            if 'ln1' in reg and not ('1' in abl and ri > 5):
                a, b = reg['ln1']
                nj = (b - a) // 16
                items += [((j * NT) // nj, ln1_task(a + 16 * j, gsel(j / nj, '1')), 0) for j in range(nj)]
            tot = sum(j[-1] for j in mm)
            acc = 0
            for job in mm:
                pos = (acc * NT) // tot
                acc += job[-1]
                if job[0] == 'qkv':
                    items.append((pos, qkv_task(*job[1:]), 1))
                else:
                    if 'att' in reg and job[1] + job[2] > reg['att'][0]:
                        pos = NT + 2
                    items.append((pos, wo_task(*job[1:]), 1))
            nl = len(ln2)
            if '2' in abl:
                ln2 = []
            for li, (a, b) in enumerate(ln2):
                nj = (b - a) // 16
                bt = reg.get('ln2batch', 1)
                off = 0
                if li * NT + 1 <= NT + 2 and any(k == 'wo' and 'att' in reg and r_ + n_ > reg['att'][0] and r_ < b and r_ + n_ > a for (k, r_, n_) in [j for j in mm if j[0] == 'wo']):
                    off = NT + 2 - li * NT
                items += [(off + li * NT + ((j // bt) * bt * NT) // nj + 1, ln2_task(a + 16 * j, gsel(j / nj, '2')), 4) for j in range(nj)]
            if 'att' in reg and 'a' not in abl:
                a, b = reg['att']
                ng = (b - a) // 8
                items += [((g * NT) // ng, attn_task(a + 8 * g, gsel(g / ng, 'a')), 3) for g in range(ng)]
            with scope(f'reg{ri:02d}'):
                run_interleaved(items, rev)

        with scope('tail'):
            bv, bi = best
            mx = jnp.max(bv, axis=0, keepdims=True)
            idxf = jnp.min(jnp.where(bv == mx, bi, 1e9), axis=0, keepdims=True)
            idxv = idxf.astype(I32)
            idx = idxv[0, 0]
            base = pl.multiple_of((idx // 16) * 16, 16)
            rows = lax.broadcasted_iota(I32, (16, D), 0)
            sel = rows == (idx - base)
            hb = x_v[pl.ds(base, 16), :].astype(F32) + _cat([att_v[c, pl.ds(base, 16), :] for c in range(NC)], 1)
            hcb = hb - jnp.sum(hb, axis=-1, keepdims=True) * (1.0 / D)
            hnb = hcb * lax.rsqrt(jnp.sum(hcb * hcb, axis=-1, keepdims=True) * (1.0 / D) + EPS)
            xs = jnp.where(sel, hnb, 0.0).astype(BF16)
            waited = [n for p in P for n in p.get('wait', [])]
            for n in ('wg', 'wu', 'wd'):
                if n not in waited:
                    dma(n).wait()
            g = jnp.dot(xs, wg_v[...], preferred_element_type=F32)
            u = jnp.dot(xs, wu_v[...], preferred_element_type=F32)
            a = (g * jax.nn.sigmoid(g) * u).astype(BF16)
            y = jnp.dot(a, wd_v[...], preferred_element_type=F32)
            gate = jax.nn.sigmoid(mx[:, 0:1])
            cur = hb + hnb
            patch_v[...] = jnp.where(sel, cur + y * gate, cur).astype(BF16)
        with scope('tail_dma'):
            for i in range(NO):
                if f'o{i}' not in waited:
                    for d in o_copy(i):
                        d.wait()
            pc = pltpu.make_async_copy(patch_v, out_hbm.at[pl.ds(base, 16), :], sem_p)
            pc.start()
            pc.wait()

    def fn(A_x, A_wqkv, A_wo, B_x, B_w_r, B_w_gate, B_w_up, B_w_down):
        del B_x
        x2 = A_x.reshape(S, D)
        anyspec = pl.BlockSpec(memory_space=pl.ANY)
        out = pl.pallas_call(
            kern,
            out_shape=jax.ShapeDtypeStruct((S, D), BF16),
            in_specs=[pl.BlockSpec(memory_space=pltpu.SMEM)] + [anyspec] * 7,
            out_specs=anyspec,
            scratch_shapes=[
                pltpu.VMEM((S, D), BF16),
                pltpu.VMEM((3, D, D), BF16),
                pltpu.VMEM((D, D), BF16),
                pltpu.VMEM((4 * NC, 320, 128), I32),
                pltpu.VMEM((NC, 960, 128), I32),
                pltpu.VMEM((NC, 320, 128), I32),
                pltpu.VMEM((NC, S // 2, 128), I32),
                pltpu.VMEM((NC, S + 16, 128), F32),
                pltpu.VMEM((NC, S + HALO, 128), F32),
                pltpu.VMEM((NC, S + HALO, 128), F32),
                pltpu.VMEM((NC, S, 128), F32),
                pltpu.VMEM((NC, S, 128), BF16) if 'c' in abl else pltpu.VMEM((S, D), BF16),
                pltpu.VMEM((NC, S, 128), F32),
                pltpu.VMEM((D, F), BF16),
                pltpu.VMEM((D, F), BF16),
                pltpu.VMEM((F, D), BF16),
                pltpu.VMEM((D,), BF16),
                pltpu.VMEM((16, D), BF16),
                pltpu.SemaphoreType.DMA((len(xgroups),)),
                pltpu.SemaphoreType.DMA((5,)),
                pltpu.SemaphoreType.DMA((3,)),
                pltpu.SemaphoreType.DMA((NO * NC,)),
                pltpu.SemaphoreType.DMA(()),
            ],
            compiler_params=pltpu.CompilerParams(vmem_limit_bytes=110 * 2 ** 20, flags=flags),
        )(np.zeros((1,), np.int32), x2, A_wqkv, A_wo, B_w_r, B_w_gate, B_w_up, B_w_down)
        return out.reshape(1, S, D)

    return fn


@jax.jit
def pallas_sequential_preLN__sliding_local_dilated__moe_arch_mod__prompt_kernel(
    A_x: jax.Array,
    A_wqkv: jax.Array,
    A_wo: jax.Array,
    B_x: jax.Array,
    B_w_r: jax.Array,
    B_w_gate: jax.Array,
    B_w_up: jax.Array,
    B_w_down: jax.Array,
):
    return make_kernel(rev=True, flags={'XLA_TPU_EVENLY_DISTRIBUTE_CRITICAL_NODES': True})(A_x, A_wqkv, A_wo, B_x, B_w_r, B_w_gate, B_w_up, B_w_down)
```

```python
import jax
import jax.numpy as jnp
from jax import lax
from jax.experimental import pallas as pl
from jax.experimental.pallas import tpu as pltpu

S, D, F = 2048, 640, 1536
H, DH, W, DIL = 32, 20, 8, 2
NC = D // 128
HALO = 16
F32 = jnp.float32
BF16 = jnp.bfloat16
I32 = jnp.int32
LOG2E = 1.4426950408889634
QSCALE = float(DH ** -0.5) * LOG2E
NEG = -1e9 * LOG2E
EPS = 1e-5


def _cat(xs, axis):
    return xs[0] if len(xs) == 1 else jnp.concatenate(xs, axis=axis)


def _regroup(src_ref, c, dp):
    a = src_ref[c, pl.ds(dp, 16, stride=20), :]
    b = src_ref[c, pl.ds(10 + dp, 16, stride=20), :]
    lo = jnp.bitwise_or(jnp.bitwise_and(a, 0xFFFF), jnp.left_shift(b, 16))
    hi = jnp.bitwise_or(lax.shift_right_logical(a, 16), jnp.bitwise_and(b, -65536))
    return lo, hi


def _bf(x):
    return pltpu.bitcast(x, BF16)


def _i32(x):
    return pltpu.bitcast(x, I32)


def run_interleaved(streams, rev=False):
    active = []
    pending = sorted(streams, key=lambda t: t[0])
    tick = 0
    while pending or active:
        while pending and pending[0][0] <= tick:
            active.append(pending.pop(0))
        active.sort(key=lambda t: (t[2], -t[0] if rev else t[0]))
        nxt = []
        for item in active:
            try:
                next(item[1])
                nxt.append(item)
            except StopIteration:
                pass
        active = nxt
        tick += 1


def default_plan():
    P = [{'ln1': (0, 128), 'wait': ['x0']},
 {'prep': ['k'], 'wait': ['wk']},
 {'ln1': (128, 384), 'mm': [('qkv', 1, 0, 128)], 'wait': ['x1']},
 {'mm': [('qkv', 1, 128, 256)], 'prep': ['v'], 'wait': ['wv']},
 {'mm': [('qkv', 2, 0, 384)], 'prep': ['q'], 'wait': ['wq', 'x2']},
 {'ln1': (384, 640), 'mm': [('qkv', 0, 0, 128), ('qkv', 0, 128, 256)], 'wait': []},
 {'att': (0, 288), 'ln1': (640, 896), 'mm': [('qkv3', 384, 256)], 'prep': ['o'], 'start': ['ffn'], 'wait': ['x3', 'wo', 'wr']},
 {'att': (288, 608), 'ln1': (896, 1152), 'mm': [('qkv3', 640, 256), ('wo', 0, 288)], 'wait': ['x4']},
 {'att': (608, 896), 'ln1': (1152, 1408), 'ln2': [(0, 288)], 'mm': [('qkv3', 896, 256), ('wo', 288, 320)], 'wait': ['x5']},
 {'att': (896, 1152), 'ln1': (1408, 1664), 'ln2': [(288, 608)], 'mm': [('qkv3', 1152, 256), ('wo', 608, 288)], 'wait': ['x6']},
 {'att': (1152, 1408), 'ln1': (1664, 1920), 'ln2': [(608, 896)], 'mm': [('qkv3', 1408, 256), ('wo', 896, 256)], 'ostart': (0, 608), 'wait': ['x7']},
 {'att': (1408, 1664),
  'ln1': (1920, 2048),
  'ln2': [(896, 1152)],
  'mm': [('qkv3', 1664, 256), ('wo', 1152, 256)],
  'ostart': (608, 896),
  'wait': ['x8']},
 {'att': (1664, 1920), 'ln2': [(1152, 1408)], 'mm': [('qkv3', 1920, 128), ('wo', 1408, 256)], 'ostart': (896, 1152), 'wait': ['wg']},
 {'att': (1920, 2048),
  'ln2': [(1408, 1664), (1664, 1920), (1920, 2048)],
  'ln2batch': 4,
  'mm': [('wo', 1664, 256), ('wo', 1920, 128)],
  'ostart': (1152, 1408),
  'wait': ['wu']},
 {'ostart': (1408, 2048)}]
    xg = [(0, 128), (128, 384), (384, 640), (640, 896), (896, 1152), (1152, 1408), (1408, 1664), (1664, 1920), (1920, 2048)]
    order = ['x0', 'wk', 'x1', 'wv', 'x2', 'wq', 'wo', 'wr', 'x3', 'x4', 'x5', 'x6', 'x7', 'x8']
    return P, xg, order


def make_kernel(rev=True):
    P, xgroups, dma_order = default_plan()
    ogroups = [p['ostart'] for p in P if 'ostart' in p]
    NO = len(ogroups)

    def kern(x_hbm, wqkv_hbm, wo_hbm, wr_hbm, wg_hbm, wu_hbm, wd_hbm, out_hbm,
             x_v, wraw, woraw, t32, wtp, wop, xn_v, q_v, k_v, v_v, att_v, out_v, o_v,
             wg_v, wu_v, wd_v, wr_v, patch_v, sem_x, sem_w, sem_f, sem_o, sem_p):
        def dma(name):
            if name[0] == 'x':
                gi = int(name[1:])
                a, b = xgroups[gi]
                return pltpu.make_async_copy(x_hbm.at[pl.ds(a, b - a), :], x_v.at[pl.ds(a, b - a), :], sem_x.at[gi])
            if name in ('wq', 'wk', 'wv'):
                p = ('wq', 'wk', 'wv').index(name)
                return pltpu.make_async_copy(wqkv_hbm.at[:, pl.ds(p * D, D)], wraw.at[p], sem_w.at[p])
            if name == 'wo':
                return pltpu.make_async_copy(wo_hbm, woraw, sem_w.at[3])
            if name == 'wr':
                return pltpu.make_async_copy(wr_hbm, wr_v, sem_w.at[4])
            if name in ('wg', 'wu', 'wd'):
                return f_copy(('wg', 'wu', 'wd').index(name))
            raise KeyError(name)

        def f_copy(i):
            return pltpu.make_async_copy((wg_hbm, wu_hbm, wd_hbm)[i], (wg_v, wu_v, wd_v)[i], sem_f.at[i])

        def o_copy(i):
            a, b = ogroups[i]
            return pltpu.make_async_copy(out_v.at[pl.ds(a, b - a), :], out_hbm.at[pl.ds(a, b - a), :], sem_o.at[i])

        for name in dma_order:
            dma(name).start()

        zeros = jnp.zeros((HALO, 128), F32)
        for c in range(NC):
            k_v[c, pl.ds(0, HALO), :] = zeros
            v_v[c, pl.ds(0, HALO), :] = zeros
        best = [jnp.full((8, 128), -jnp.inf, F32), jnp.zeros((8, 128), F32)]

        def prep_w(p):
            for kt in range(NC):
                for ft in range(NC):
                    tile = wraw[p, pl.ds(kt * 128, 128), pl.ds(ft * 128, 128)]
                    t32[p * NC + kt, pl.ds(64 * ft, 64), :] = _i32(tile.T)
            for kt in range(NC):
                for dp in range(10):
                    lo, hi = _regroup(t32, p * NC + kt, dp)
                    wtp[kt, pl.ds(p * 320 + 32 * dp, 16), :] = lo
                    wtp[kt, pl.ds(p * 320 + 32 * dp + 16, 16), :] = hi

        def prep_wo():
            for c in range(NC):
                t32[3 * NC + c] = _i32(woraw[:, pl.ds(c * 128, 128)])
            for c in range(NC):
                for dp in range(10):
                    lo, hi = _regroup(t32, 3 * NC + c, dp)
                    wop[c, pl.ds(32 * dp, 16), :] = lo
                    wop[c, pl.ds(32 * dp + 16, 16), :] = hi

        def load_bf(ref, c, r, n):
            return _bf(ref[c, pl.ds(r // 2, n // 2), :])

        done = {k: set() for k in ('x', 'xn', 0, 1, 2, 'o', 'att', 'out')}

        def need(k, a, b):
            assert all(r in done[k] for r in range(max(a, 0), b)), (k, a, b)

        def mark(k, a, b):
            done[k].update(range(a, b))

        def ln1_task(r):
            need('x', r, r + 16)
            xf = x_v[pl.ds(r, 16), :].astype(F32)
            m = jnp.sum(xf, axis=-1, keepdims=True) * (1.0 / D)
            yield
            xc = xf - m
            v = jnp.sum(xc * xc, axis=-1, keepdims=True) * (1.0 / D)
            yield
            xn = (xc * lax.rsqrt(v + EPS)).astype(BF16)
            for c in range(NC):
                xn_v[c, pl.ds(r // 2, 8), :] = _i32(xn[:, c * 128:(c + 1) * 128])
            mark('xn', r, r + 16)

        def qkv_task(p, r, n):
            need('xn', r, r + n)
            mark(p, r, r + n)
            lhs = _cat([load_bf(xn_v, c, r, n) for c in range(NC)], 1)
            rhs = _cat([load_bf(wtp, c, p * D, D) for c in range(NC)], 1)
            y = lax.dot_general(lhs, rhs, (((1,), (1,)), ((), ())), preferred_element_type=F32)
            for c in range(NC):
                yc = y[:, c * 128:(c + 1) * 128]
                if p == 0:
                    q_v[c, pl.ds(r, n), :] = yc * QSCALE
                elif p == 1:
                    k_v[c, pl.ds(HALO + r, n), :] = yc
                else:
                    v_v[c, pl.ds(HALO + r, n), :] = yc
            yield

        def attn_task(r):
            need(0, r, r + 8)
            need(1, r - 14, r + 8)
            need(2, r - 14, r + 8)
            q = [q_v[c, pl.ds(r, 8), :] for c in range(NC)]
            s = []
            for w in range(W):
                acc = None
                for c in range(NC):
                    pr = q[c] * k_v[c, pl.ds(HALO + r - DIL * w, 8), :]
                    acc = pr if acc is None else acc + pr
                s.append(acc)
            rr = [pltpu.roll(a, 64, 1) for a in s]
            yield
            s = [a + b for a, b in zip(s, rr)]
            rr = [pltpu.roll(a, 32, 1) for a in s]
            yield
            s = [a + b for a, b in zip(s, rr)]
            for w in range(W):
                if r < DIL * w:
                    rows = r + lax.broadcasted_iota(I32, (8, 128), 0)
                    s[w] = jnp.where(rows >= DIL * w, s[w], NEG)
            m = s[0]
            for w in range(1, W):
                m = jnp.maximum(m, s[w])
            p = [jnp.exp2(s[w] - m) for w in range(W)]
            l = p[0]
            for w in range(1, W):
                l = l + p[w]
            y0 = pl.reciprocal(l, approx=True)
            inv = y0 * (2.0 - l * y0)
            for c in range(NC):
                acc = None
                for w in range(W):
                    pr = p[w] * v_v[c, pl.ds(HALO + r - DIL * w, 8), :]
                    acc = pr if acc is None else acc + pr
                o_v[c, pl.ds(r, 8), :] = acc * inv
            mark('o', r, r + 8)

        def wo_task(r, n):
            need('o', r, r + n)
            mark('att', r, r + n)
            lhs = _cat([o_v[c, pl.ds(r, n), :].astype(BF16) for c in range(NC)], 1)
            rhs = _cat([load_bf(wop, c, 0, D) for c in range(NC)], 1)
            y = jnp.dot(lhs, rhs, preferred_element_type=F32)
            for c in range(NC):
                att_v[c, pl.ds(r, n), :] = y[:, c * 128:(c + 1) * 128]
            yield

        def ln2_task(r):
            need('att', r, r + 16)
            att = [att_v[c, pl.ds(r, 16), :] for c in range(NC)]
            att = _cat(att, 1)
            h = x_v[pl.ds(r, 16), :].astype(F32) + att
            m = jnp.sum(h, axis=-1, keepdims=True) * (1.0 / D)
            yield
            hc = h - m
            v = jnp.sum(hc * hc, axis=-1, keepdims=True) * (1.0 / D)
            yield
            hn = hc * lax.rsqrt(v + EPS)
            wr = wr_v[...].astype(F32).reshape(1, D)
            rr = jnp.sum(hn * wr, axis=-1, keepdims=True)
            ob = (h + hn).astype(BF16)
            out_v[pl.ds(r, 16), :] = ob
            mark('out', r, r + 16)
            yield
            for g in range(2):
                rg = jnp.broadcast_to(rr[8 * g:8 * g + 8], (8, 128))
                idx = (r + 8 * g + lax.broadcasted_iota(I32, (8, 128), 0)).astype(F32)
                bv, bi = best
                better = rg > bv
                best[0] = jnp.where(better, rg, bv)
                best[1] = jnp.where(better, idx, bi)

        def call_task(f, *a):
            f(*a)
            yield

        oi = 0
        for reg in P:
            for name in reg.get('wait', []):
                dma(name).wait()
                if name[0] == 'x':
                    mark('x', *xgroups[int(name[1:])])
            if 'ffn' in reg.get('start', []):
                for i in range(3):
                    f_copy(i).start()
            if 'ostart' in reg:
                need('out', *reg['ostart'])
                o_copy(oi).start()
                oi += 1
            mm = []
            for job in reg.get('mm', []):
                if job[0] == 'qkv3':
                    mm += [('qkv', p, job[1], job[2]) for p in (1, 2, 0)]
                else:
                    mm.append(job)
            NT = max(1, sum(j[-1] for j in mm) // 32)
            ln2 = reg.get('ln2', [])
            NT = max([NT] + [(reg[k][1] - reg[k][0]) // 8 for k in ('ln1', 'att') if k in reg] + [(b - a) // 8 for a, b in ln2])
            items = []
            for pn in reg.get('prep', []):
                items.append((0, call_task(prep_wo) if pn == 'o' else call_task(prep_w, 'qkv'.index(pn)), 9))
            if 'ln1' in reg:
                a, b = reg['ln1']
                nj = (b - a) // 16
                items += [((j * NT) // nj, ln1_task(a + 16 * j), 0) for j in range(nj)]
            tot = sum(j[-1] for j in mm)
            acc = 0
            for job in mm:
                pos = (acc * NT) // tot
                acc += job[-1]
                if job[0] == 'qkv':
                    items.append((pos, qkv_task(*job[1:]), 1))
                else:
                    if 'att' in reg and job[1] + job[2] > reg['att'][0]:
                        pos = NT + 2
                    items.append((pos, wo_task(*job[1:]), 1))
            for li, (a, b) in enumerate(ln2):
                nj = (b - a) // 16
                bt = reg.get('ln2batch', 1)
                off = 0
                if li * NT + 1 <= NT + 2 and any(k == 'wo' and 'att' in reg and r_ + n_ > reg['att'][0] and r_ < b and r_ + n_ > a for (k, r_, n_) in [j for j in mm if j[0] == 'wo']):
                    off = NT + 2 - li * NT
                items += [(off + li * NT + ((j // bt) * bt * NT) // nj + 1, ln2_task(a + 16 * j), 4) for j in range(nj)]
            if 'att' in reg:
                a, b = reg['att']
                ng = (b - a) // 8
                items += [((g * NT) // ng, attn_task(a + 8 * g), 3) for g in range(ng)]
            run_interleaved(items, rev)

        bv, bi = best
        mx = jnp.max(bv, axis=0, keepdims=True)
        idxf = jnp.min(jnp.where(bv == mx, bi, 1e9), axis=0, keepdims=True)
        idxv = idxf.astype(I32)
        idx = idxv[0, 0]
        base = pl.multiple_of(jnp.clip((idx // 16) * 16, 0, S - 16), 16)
        rows = lax.broadcasted_iota(I32, (16, D), 0)
        sel = rows == (idx - base)
        hb = x_v[pl.ds(base, 16), :].astype(F32) + _cat([att_v[c, pl.ds(base, 16), :] for c in range(NC)], 1)
        hcb = hb - jnp.sum(hb, axis=-1, keepdims=True) * (1.0 / D)
        hnb = hcb * lax.rsqrt(jnp.sum(hcb * hcb, axis=-1, keepdims=True) * (1.0 / D) + EPS)
        xs = jnp.where(sel, hnb, 0.0).astype(BF16)
        waited = [n for p in P for n in p.get('wait', [])]
        for n in ('wg', 'wu', 'wd'):
            if n not in waited:
                dma(n).wait()
        g = jnp.dot(xs, wg_v[...], preferred_element_type=F32)
        u = jnp.dot(xs, wu_v[...], preferred_element_type=F32)
        a = (g * jax.nn.sigmoid(g) * u).astype(BF16)
        y = jnp.dot(a, wd_v[...], preferred_element_type=F32)
        gate = jax.nn.sigmoid(mx[:, 0:1])
        cur = hb + hnb
        patch_v[...] = jnp.where(sel, cur + y * gate, cur).astype(BF16)
        for i in range(NO):
            o_copy(i).wait()
        pc = pltpu.make_async_copy(patch_v, out_hbm.at[pl.ds(base, 16), :], sem_p)
        pc.start()
        pc.wait()

    def fn(A_x, A_wqkv, A_wo, B_x, B_w_r, B_w_gate, B_w_up, B_w_down):
        del B_x
        x2 = A_x.reshape(S, D)
        anyspec = pl.BlockSpec(memory_space=pl.ANY)
        out = pl.pallas_call(
            kern,
            out_shape=jax.ShapeDtypeStruct((S, D), BF16),
            in_specs=[anyspec] * 7,
            out_specs=anyspec,
            scratch_shapes=[
                pltpu.VMEM((S, D), BF16),
                pltpu.VMEM((3, D, D), BF16),
                pltpu.VMEM((D, D), BF16),
                pltpu.VMEM((4 * NC, 320, 128), I32),
                pltpu.VMEM((NC, 960, 128), I32),
                pltpu.VMEM((NC, 320, 128), I32),
                pltpu.VMEM((NC, S // 2, 128), I32),
                pltpu.VMEM((NC, S + 16, 128), F32),
                pltpu.VMEM((NC, S + HALO, 128), F32),
                pltpu.VMEM((NC, S + HALO, 128), F32),
                pltpu.VMEM((NC, S, 128), F32),
                pltpu.VMEM((S, D), BF16),
                pltpu.VMEM((NC, S, 128), F32),
                pltpu.VMEM((D, F), BF16),
                pltpu.VMEM((D, F), BF16),
                pltpu.VMEM((F, D), BF16),
                pltpu.VMEM((D,), BF16),
                pltpu.VMEM((16, D), BF16),
                pltpu.SemaphoreType.DMA((len(xgroups),)),
                pltpu.SemaphoreType.DMA((5,)),
                pltpu.SemaphoreType.DMA((3,)),
                pltpu.SemaphoreType.DMA((NO,)),
                pltpu.SemaphoreType.DMA(()),
            ],
            compiler_params=pltpu.CompilerParams(vmem_limit_bytes=110 * 2 ** 20, flags={'XLA_TPU_EVENLY_DISTRIBUTE_CRITICAL_NODES': True}),
        )(x2, A_wqkv, A_wo, B_w_r, B_w_gate, B_w_up, B_w_down)
        return out.reshape(1, S, D)

    return fn


@jax.jit
def pallas_sequential_preLN__sliding_local_dilated__moe_arch_mod__prompt_kernel(
    A_x: jax.Array,
    A_wqkv: jax.Array,
    A_wo: jax.Array,
    B_x: jax.Array,
    B_w_r: jax.Array,
    B_w_gate: jax.Array,
    B_w_up: jax.Array,
    B_w_down: jax.Array,
):
    return make_kernel()(A_x, A_wqkv, A_wo, B_x, B_w_r, B_w_gate, B_w_up, B_w_down)
```
